```python
import jax
import jax.numpy as jnp

def _softmax(x, axis=-1):
    return jax.nn.softmax(x, axis=axis)
def _gelu(x):
    return jax.nn.gelu(x, approximate=True)
def _silu(x):
    return jax.nn.silu(x)
def _sigmoid(x):
    return jax.nn.sigmoid(x)
def _layernorm(x, axis=-1, eps=1e-5):
    m = jnp.mean(x, axis=axis, keepdims=True)
    v = jnp.var(x, axis=axis, keepdims=True)
    return (x - m) / jnp.sqrt(v + eps)
def _scatter_add(tgt, idx, src, axis=0):
    return tgt.at[idx].add(src)
def _segment_sum(src, seg, n):
    return jax.ops.segment_sum(src, seg, n)
class _Rng:
    def __init__(self, key):
        self._k = key
    def _next(self):
        self._k, sub = jax.random.split(self._k)
        return sub
    def normal(self, shape):
        return jax.random.normal(self._next(), shape, dtype=jnp.bfloat16)
    def randint(self, lo, hi, shape):
        return jax.random.randint(self._next(), shape, lo, hi, dtype=jnp.int32)
    def uniform(self, shape, lo=0.0, hi=1.0):
        return jax.random.uniform(self._next(), shape, jnp.bfloat16, lo, hi)
    def permutation(self, n):
        return jax.random.permutation(self._next(), n)


kernel_name = 'standalone__detection_seg_fpn_lateral__vision'

def setup_inputs():
    _rng = _Rng(jax.random.key(int.from_bytes(__import__("os").urandom(4), "little")))
    _w = (lambda a: (lambda t: t.astype(jnp.bfloat16) if jnp.issubdtype(t.dtype, jnp.floating) else t)(jnp.asarray(a)))
    H = W = (384 // 2) * 2
    C = 384
    k = 1
    return {
        "c_fine": _w((lambda *s: _rng.normal(s) * 0.05)(1, H, W, C)),
        "p_coarse": _w((lambda *s: _rng.normal(s) * 0.05)(1, H // 2, W // 2, C)),
        "w_lat": _w((lambda *s: _rng.normal(s) * 0.05)(C, C)),
        "w_out": _w((lambda *s: _rng.normal(s) * 0.05)(k, k, C, C)),
    }

def reference(c_fine, p_coarse, w_lat, w_out):
    B, H, W, C = c_fine.shape
    k = 1
    lat = jnp.einsum("bhwc,cd->bhwd", c_fine, w_lat)
    up = jnp.repeat(jnp.repeat(p_coarse, 2, axis=1), 2, axis=2)
    m = lat + up
    pad = k // 2
    mp = jnp.pad(m, ((0, 0), (pad, pad), (pad, pad), (0, 0)))
    o = None
    for di in range(k):
        for dj in range(k):
            t = jnp.einsum("bhwc,cd->bhwd", mp[:, di:di + H, dj:dj + W, :], w_out[di, dj])
            o = t if o is None else o + t
    return o
```

```python
import jax
import jax.numpy as jnp
import jax.experimental.pallas as pl
import jax.experimental.pallas.tpu as pltpu


@jax.jit
def pallas_standalone__detection_seg_fpn_lateral__vision_kernel(
    c_fine: jax.Array,
    p_coarse: jax.Array,
    w_lat: jax.Array,
    w_out: jax.Array,
):
    B, H, W, C = c_fine.shape
    bh = 8
    c2 = c_fine.reshape(B * H * W, C)
    p2 = p_coarse.reshape(B * (H // 2) * (W // 2), C)
    wo = w_out.reshape(C, C)

    def kernel_function(c_ref, p_ref, wl_ref, wo_ref, o_ref, w_ref):
        @pl.when(pl.program_id(0) == 0)
        def _():
            w_ref[...] = jnp.dot(
                wl_ref[...], wo_ref[...], preferred_element_type=jnp.float32
            ).astype(jnp.bfloat16)

        for r in range(bh // 2):
            q = jnp.dot(
                p_ref[r * (W // 2):(r + 1) * (W // 2), :],
                wo_ref[...],
                preferred_element_type=jnp.float32,
            )
            qq = pltpu.pack_elementwise([q, q], packed_dtype=jnp.bfloat16)
            qu = pltpu.bitcast(qq, jnp.bfloat16).astype(jnp.float32)
            for s in range(2):
                rows = slice((2 * r + s) * W, (2 * r + s + 1) * W)
                y = jnp.dot(c_ref[rows, :], w_ref[...], preferred_element_type=jnp.float32)
                o_ref[rows, :] = (y + qu).astype(jnp.bfloat16)

    out = pl.pallas_call(
        kernel_function,
        grid=(B * H // bh,),
        in_specs=[
            pl.BlockSpec((bh * W, C), lambda i: (i, 0)),
            pl.BlockSpec((bh // 2 * W // 2, C), lambda i: (i, 0)),
            pl.BlockSpec((C, C), lambda i: (0, 0)),
            pl.BlockSpec((C, C), lambda i: (0, 0)),
        ],
        out_specs=pl.BlockSpec((bh * W, C), lambda i: (i, 0)),
        out_shape=jax.ShapeDtypeStruct((B * H * W, C), jnp.bfloat16),
        scratch_shapes=[pltpu.VMEM((C, C), jnp.bfloat16)],
        compiler_params=pltpu.CompilerParams(
            dimension_semantics=("arbitrary",), vmem_limit_bytes=64 << 20
        ),
    )(c2, p2, w_lat, wo)
    return out.reshape(B, H, W, C)
```

```python
import jax
import jax.numpy as jnp
from jax import lax
import jax.experimental.pallas as pl
import jax.experimental.pallas.tpu as pltpu

STREAMS = 8
UNIT_W = 96
RUN_W = 48
PHASE_UNITS = 24
FLIP_AT = 13


def _upsample_rows(q):
    u = pltpu.bitcast(q.astype(jnp.bfloat16).astype(jnp.float32), jnp.uint32)
    return pltpu.bitcast(u | (u >> 16), jnp.bfloat16).astype(jnp.float32)


def _loop(lo, hi, fn):
    def body(i, carry):
        fn(i)
        return carry

    lax.fori_loop(lo, hi, body, None)


def _start(copies):
    for c in copies:
        c.start()


def _wait(copies):
    for c in copies:
        c.wait()


@jax.jit
def pallas_standalone__detection_seg_fpn_lateral__vision_kernel(
    c_fine: jax.Array,
    p_coarse: jax.Array,
    w_lat: jax.Array,
    w_out: jax.Array,
):
    B, H, W, C = c_fine.shape
    A, wu, R, U, F = STREAMS, UNIT_W, RUN_W, PHASE_UNITS, FLIP_AT
    pairs = B * H // 2 // A
    units_per_row = W // wu
    n_units = pairs * units_per_row
    n_phases = n_units // U
    runs = wu // R
    assert w_out.shape[:2] == (1, 1)
    assert pairs * A * 2 == B * H and units_per_row * wu == W and n_phases * U == n_units

    def kernel_function(c_hbm, p_hbm, wl_hbm, wo_hbm, o_hbm,
                        cbuf, pbuf, obuf, wl_ref, wo_ref, w_ref, rsem, wsem, csem):
        def reads(u, s):
            b, j = u // units_per_row, lax.rem(u, units_per_row)
            pc = pl.ds(pl.multiple_of(j * (wu // 2), wu // 2), wu // 2)
            fc = pl.ds(pl.multiple_of(j * wu, wu), wu)
            return [
                pltpu.make_async_copy(p_hbm.at[:, b, pc], pbuf.at[s], rsem.at[s]),
                pltpu.make_async_copy(c_hbm.at[:, b, :, fc], cbuf.at[s], rsem.at[s]),
            ]

        def writes(u, s):
            b, j = u // units_per_row, lax.rem(u, units_per_row)
            return [
                pltpu.make_async_copy(
                    obuf.at[s, par, :, pl.ds(h * R, R)],
                    o_hbm.at[:, b, par, pl.ds(pl.multiple_of(j * wu + h * R, R), R)],
                    wsem.at[s, int(par == 1 and h == runs - 1)],
                )
                for par in range(2)
                for h in range(runs)
            ]

        weights = [
            pltpu.make_async_copy(wl_hbm, wl_ref, csem.at[0]),
            pltpu.make_async_copy(wo_hbm, wo_ref, csem.at[1]),
        ]
        _start(weights)
        _loop(0, U, lambda t: _start(reads(t, t)))
        _wait(weights)
        w_ref[...] = jnp.dot(
            wl_ref[...], wo_ref[...], preferred_element_type=jnp.float32
        ).astype(jnp.bfloat16)

        def unit(u):
            phase, s = u // U, lax.rem(u, U)
            base = phase * U

            @pl.when(s == F)
            def _():
                _loop(F, U - 1, lambda t: _wait(reads(base + t, t)))
                _loop(0, F, lambda t: _start(writes(base + t, t)))

            @pl.when(jnp.logical_or(s < F, s == U - 1))
            def _():
                _wait(reads(u, s))

            q = jnp.dot(pbuf[s].reshape(A * wu // 2, C), wo_ref[...],
                        preferred_element_type=jnp.float32)
            up = _upsample_rows(q)
            for par in range(2):
                y = jnp.dot(cbuf[s, :, par].reshape(A * wu, C), w_ref[...],
                            preferred_element_type=jnp.float32)
                obuf[s, par] = (y + up).astype(jnp.bfloat16).reshape(A, wu, C)

            @pl.when(s >= F)
            def _():
                _start(writes(u, s))

            @pl.when(s == U - 1)
            def _():
                _loop(0, U - 1, lambda t: _wait(writes(base + t, t)))
                last = writes(u, s)
                _wait(last[:-1])

                @pl.when(phase + 1 < n_phases)
                def _():
                    _loop(0, U, lambda t: _start(reads(base + U + t, t)))

                _wait(last[-1:])

        _loop(0, n_units, unit)

    out = pl.pallas_call(
        kernel_function,
        in_specs=[pl.BlockSpec(memory_space=pl.ANY)] * 4,
        out_specs=pl.BlockSpec(memory_space=pl.ANY),
        out_shape=jax.ShapeDtypeStruct((A, pairs, 2, W, C), c_fine.dtype),
        scratch_shapes=[
            pltpu.VMEM((U, A, 2, wu, C), jnp.bfloat16),
            pltpu.VMEM((U, A, wu // 2, C), jnp.bfloat16),
            pltpu.VMEM((U, 2, A, wu, C), jnp.bfloat16),
            pltpu.VMEM((C, C), jnp.bfloat16),
            pltpu.VMEM((C, C), jnp.bfloat16),
            pltpu.VMEM((C, C), jnp.bfloat16),
            pltpu.SemaphoreType.DMA((U,)),
            pltpu.SemaphoreType.DMA((U, 2)),
            pltpu.SemaphoreType.DMA((2,)),
        ],
        compiler_params=pltpu.CompilerParams(vmem_limit_bytes=100 << 20),
    )(
        c_fine.reshape(A, pairs, 2, W, C),
        p_coarse.reshape(A, pairs, W // 2, C),
        w_lat,
        w_out.reshape(C, C),
    )
    return out.reshape(B, H, W, C)
```

```python
import jax
import jax.numpy as jnp
from jax import lax
import jax.experimental.pallas as pl
import jax.experimental.pallas.tpu as pltpu

BANDS = 8
UNIT_W = 96
RUN_W = 48
PHASE_UNITS = 32
FLIP_AT = 19


def _repeat_rows(q):
    u = pltpu.bitcast(q.astype(jnp.bfloat16).astype(jnp.float32), jnp.uint32)
    return pltpu.bitcast(u | (u >> 16), jnp.bfloat16).astype(jnp.float32)


def _loop(lo, hi, fn):
    def body(i, carry):
        fn(i)
        return carry

    lax.fori_loop(lo, hi, body, None)


def _start(copies):
    for copy in copies:
        copy.start()


def _wait(copies):
    for copy in copies:
        copy.wait()


@jax.jit
def pallas_standalone__detection_seg_fpn_lateral__vision_kernel(
    c_fine: jax.Array,
    p_coarse: jax.Array,
    w_lat: jax.Array,
    w_out: jax.Array,
):
    B, H, W, C = c_fine.shape
    A, U, F = BANDS, PHASE_UNITS, FLIP_AT
    pairs = B * H // (2 * A)
    row_units = W // UNIT_W
    row_runs = W // RUN_W
    unit_runs = UNIT_W // RUN_W
    n_units = pairs * row_units
    n_rounds = n_units // U
    T = U * 2 * unit_runs
    assert w_out.shape == (1, 1, C, C)
    assert pairs * 2 * A == B * H and row_units * UNIT_W == W
    assert n_rounds * U == n_units and U % row_units == 0

    def kernel_function(c_hbm, p_hbm, wl_hbm, wo_hbm, o_hbm,
                        c_buf, p_buf, o_buf, wl_ref, wo_ref, w_ref,
                        read_sems, write_sems, weight_sems):
        def reads(rnd, s):
            pair = rnd * (U // row_units) + s // row_units
            j = s % row_units
            fine = pl.ds(pl.multiple_of(j * UNIT_W, UNIT_W), UNIT_W)
            coarse = pl.ds(pl.multiple_of(j * (UNIT_W // 2), UNIT_W // 2), UNIT_W // 2)
            return [
                pltpu.make_async_copy(c_hbm.at[:, pair, :, fine], c_buf.at[s], read_sems.at[s, 0]),
                pltpu.make_async_copy(p_hbm.at[:, pair, coarse], p_buf.at[s], read_sems.at[s, 1]),
            ]

        def write(rnd, t, sem=0):
            return pltpu.make_async_copy(o_buf.at[t], o_hbm.at[:, rnd * T + t], write_sems.at[sem])

        def done_runs(s):
            return (s // row_units) * 2 * row_runs + (s % row_units) * unit_runs

        def start_reads(rnd):
            _loop(0, U, lambda s: _start(reads(rnd, s)))

        weights = [
            pltpu.make_async_copy(wl_hbm, wl_ref, weight_sems.at[0]),
            pltpu.make_async_copy(wo_hbm, wo_ref, weight_sems.at[1]),
        ]
        _start(weights)
        start_reads(0)
        _wait(weights)
        w_ref[...] = jnp.dot(
            wl_ref[...], wo_ref[...], preferred_element_type=jnp.float32
        ).astype(w_ref.dtype)

        def unit(u):
            rnd, s = lax.div(u, U), lax.rem(u, U)

            @pl.when(s < F)
            def _():
                _wait(reads(rnd, s))

            @pl.when(s == F)
            def _():
                _loop(F, U - 1, lambda i: _wait(reads(rnd, i)))
                last_c, last_p = reads(rnd, U - 1)
                last_c.wait()
                _loop(0, done_runs(F), lambda t: write(rnd, t).start())
                last_p.wait()

            q = jnp.dot(p_buf[s].reshape(A * UNIT_W // 2, C), wo_ref[...],
                        preferred_element_type=jnp.float32)
            up = _repeat_rows(q)
            for row in range(2):
                y = jnp.dot(c_buf[s, :, row].reshape(A * UNIT_W, C), w_ref[...],
                            preferred_element_type=jnp.float32)
                o = (y + up).astype(o_buf.dtype).reshape(A, unit_runs, RUN_W, C)
                for h in range(unit_runs):
                    o_buf[done_runs(s) + row * row_runs + h] = o[:, h]

            @pl.when(s >= F)
            def _():
                _loop(done_runs(s), jnp.minimum(done_runs(s + 1), T - 1),
                      lambda t: write(rnd, t).start())

            @pl.when(s == U - 1)
            def _():
                write(rnd, T - 1, sem=1).start()
                _loop(0, T - 1, lambda t: write(rnd, t).wait())

                @pl.when(rnd + 1 < n_rounds)
                def _():
                    start_reads(rnd + 1)

                write(rnd, T - 1, sem=1).wait()

        _loop(0, n_units, unit)

    out = pl.pallas_call(
        kernel_function,
        in_specs=[pl.BlockSpec(memory_space=pl.ANY)] * 4,
        out_specs=pl.BlockSpec(memory_space=pl.ANY),
        out_shape=jax.ShapeDtypeStruct((A, pairs * 2 * row_runs, RUN_W, C), c_fine.dtype),
        scratch_shapes=[
            pltpu.VMEM((U, A, 2, UNIT_W, C), c_fine.dtype),
            pltpu.VMEM((U, A, UNIT_W // 2, C), p_coarse.dtype),
            pltpu.VMEM((T, A, RUN_W, C), c_fine.dtype),
            pltpu.VMEM((C, C), w_lat.dtype),
            pltpu.VMEM((C, C), w_out.dtype),
            pltpu.VMEM((C, C), c_fine.dtype),
            pltpu.SemaphoreType.DMA((U, 2)),
            pltpu.SemaphoreType.DMA((2,)),
            pltpu.SemaphoreType.DMA((2,)),
        ],
        compiler_params=pltpu.CompilerParams(vmem_limit_bytes=110 << 20),
    )(
        c_fine.reshape(A, pairs, 2, W, C),
        p_coarse.reshape(A, pairs, W // 2, C),
        w_lat,
        w_out.reshape(C, C),
    )
    return out.reshape(B, H, W, C)
```
